```python
import os as _os
_os.environ.setdefault("JAX_PLATFORMS", "cpu")
import jax
import jax.numpy as jnp

def _softmax(x, axis=-1):
    return jax.nn.softmax(x, axis=axis)
def _gelu(x):
    return jax.nn.gelu(x, approximate=True)
def _silu(x):
    return jax.nn.silu(x)
def _sigmoid(x):
    return jax.nn.sigmoid(x)
def _layernorm(x, axis=-1, eps=1e-5):
    m = jnp.mean(x, axis=axis, keepdims=True)
    v = jnp.var(x, axis=axis, keepdims=True)
    return (x - m) / jnp.sqrt(v + eps)
def _scatter_add(tgt, idx, src, axis=0):
    return tgt.at[idx].add(src)
def _segment_sum(src, seg, n):
    return jax.ops.segment_sum(src, seg, n)
class _Rng:
    def __init__(self, key):
        self._k = key
    def _next(self):
        self._k, sub = jax.random.split(self._k)
        return sub
    def normal(self, shape):
        return jax.random.normal(self._next(), shape, dtype=jnp.bfloat16)
    def randint(self, lo, hi, shape):
        return jax.random.randint(self._next(), shape, lo, hi, dtype=jnp.int32)
    def uniform(self, shape, lo=0.0, hi=1.0):
        return jax.random.uniform(self._next(), shape, jnp.bfloat16, lo, hi)
    def permutation(self, n):
        return jax.random.permutation(self._next(), n)


kernel_name = 'parallel_sum__mha_block__swiglu_ffn__prompt'

def setup_inputs():
    _rng = _Rng(jax.random.key(int.from_bytes(__import__("os").urandom(4), "little")))
    _w = (lambda a: (lambda t: t.astype(jnp.bfloat16) if jnp.issubdtype(t.dtype, jnp.floating) else t)(jnp.asarray(a)))
    def _A_setup():
        B, S, D, H = 1, 2048, 512, 32
        return {
            "x": _w((lambda *s: _rng.normal(s) * 0.05)(B, S, D)),
            "wqkv": _w((lambda *s: _rng.normal(s) * 0.1)(D, 3 * D)),
            "wo": _w((lambda *s: _rng.normal(s) * 0.05)(D, D)),
        }
    _A_in = _A_setup()

    def _B_setup():
        B, S, D, F = 1, 2048, 512, 1792
        return {
            "x": _w((lambda *s: _rng.normal(s) * 0.05)(B, S, D)),
            "w_gate": _w((lambda *s: _rng.normal(s) * 0.05)(D, F)),
            "w_up": _w((lambda *s: _rng.normal(s) * 0.05)(D, F)),
            "w_down": _w((lambda *s: _rng.normal(s) * 0.05)(F, D)),
        }
    _B_in = _B_setup()

    return {
        "A_x": _A_in["x"],
        "A_wqkv": _A_in["wqkv"],
        "A_wo": _A_in["wo"],
        "B_x": _B_in["x"],
        "B_w_gate": _B_in["w_gate"],
        "B_w_up": _B_in["w_up"],
        "B_w_down": _B_in["w_down"],
    }

def reference(A_x, A_wqkv, A_wo, B_x, B_w_gate, B_w_up, B_w_down):
    def _A_ref(x, wqkv, wo):
        B, S, D = x.shape
        H = 32
        Dh = D // H
        qkv = (lambda x, *d: x.transpose(*d))((x @ wqkv).reshape(B, S, 3, H, Dh), 2, 0, 3, 1, 4)
        q, k, v = qkv[0], qkv[1], qkv[2]
        scores = jnp.einsum("bhqd,bhkd->bhqk", q, k) * (Dh ** -0.5)
        p = _softmax(scores, axis=-1)
        o = jnp.einsum("bhqk,bhkd->bhqd", p, v)
        return (lambda x, *d: x.transpose(*d))(o, 0, 2, 1, 3).reshape(B, S, D) @ wo

    def _B_ref(x, w_gate, w_up, w_down):
        g = _silu(x @ w_gate)
        u = x @ w_up
        return (g * u) @ w_down

    x = A_x
    xn = _layernorm(x, axis=-1)
    return x + _A_ref(xn, A_wqkv, A_wo) + _B_ref(xn, B_w_gate, B_w_up, B_w_down)
```

```python
import jax, jax.numpy as jnp
import jax.experimental.pallas as pl
import jax.experimental.pallas.tpu as pltpu
S, D, H, DH, F = 2048, 512, 32, 16, 1792
BQ = 512
f32, bf16 = jnp.float32, jnp.bfloat16

def _ln(x):
    x = x.astype(f32)
    m = jnp.mean(x, axis=-1, keepdims=True)
    c = x - m
    v = jnp.mean(c * c, axis=-1, keepdims=True)
    return c * jax.lax.rsqrt(v + 1e-5)

CH = 128
LAG = 4
SK = 0
R = 256
U = 2
def kern(x_h, wqkv_h, wo_h, wg_h, wu_h, wd_h, o_ref, x_ref, wqkv_ref, wo_ref, wg_ref, wu_ref, wd_ref,
         xn_s, k_s, qt_s, vt_s, ot_s, sa, sb, xsem, wsem):
    i = pl.program_id(0)
    wc = [pltpu.make_async_copy(a, b, wsem.at[j]) for j, (a, b) in enumerate(
        ((wqkv_h, wqkv_ref), (wo_h, wo_ref), (wg_h, wg_ref), (wu_h, wu_ref), (wd_h, wd_ref)))]
    @pl.when(i == 0)
    def _():
        xc = [pltpu.make_async_copy(x_h.at[pl.ds(r * R, R)], x_ref.at[pl.ds(r * R, R)], xsem.at[r]) for r in range(S // R)]
        xc[0].start()
        wc[0].start()
        for c in xc[1:] + wc[1:]:
            c.start()
        wc[0].wait()
        for r in range(S // R):
            rows = pl.ds(r * R, R)
            xc[r].wait()
            xn = _ln(x_ref[rows, :]).astype(bf16)
            xn_s[rows, :] = xn
            qkv = jnp.dot(xn, wqkv_ref[...], preferred_element_type=f32)
            q = qkv[:, :D] * (0.25 * 1.4426950408889634)
            qt = q.T.astype(bf16)
            kk = pltpu.bitcast(qkv[:, D:2 * D].astype(bf16), jnp.int32)
            vt = pltpu.bitcast(qkv[:, 2 * D:].T.astype(bf16), jnp.int32)
            for h in range(H):
                qt_s[h, :, rows] = qt[h * DH:(h + 1) * DH]
                k_s[h, pl.ds(r * R // 2, R // 2), :] = kk[:, h * DH:(h + 1) * DH]
                vt_s[h, :, rows] = vt[h * 8:(h + 1) * 8]
    q0 = pl.multiple_of(i * BQ, BQ)

    def stage(hq, s_w, hp, s_r, m_cur):
        if hq is not None:
            qh = qt_s[hq, :, pl.ds(q0, BQ)]
        mx = None
        acc = None
        ts = []
        ls = None
        NC = S // CH
        for cc in range(NC + SK):
            ks = pl.ds(cc * CH, CH)
            if hq is not None and cc < NC:
                s = jnp.dot(pltpu.bitcast(k_s[hq, pl.ds(cc * CH // 2, CH // 2), :], bf16), qh, preferred_element_type=f32)
                s_w[ks, :] = s
                t = jnp.max(s.reshape(CH // 8, 8, BQ), axis=0)
                mx = t if mx is None else jnp.maximum(mx, t)
                ts.append(mx)
            c = cc - SK
            ks = pl.ds(c * CH, CH)
            if hp is not None and c >= 0:
                mc = m_cur
                if hq is not None and cc >= LAG:
                    mc = jnp.maximum(m_cur, jnp.minimum(ts[cc - LAG], m_cur))
                pf = jnp.exp2((s_r[ks, :].reshape(CH // 8, 8, BQ) - mc).reshape(CH, BQ))
                t = jnp.sum(pf.reshape(CH // 8, 8, BQ), axis=0)
                ls = t if ls is None else ls + t
                p = pf.astype(bf16)
                o = jnp.dot(pltpu.bitcast(vt_s[hp, :, ks], bf16), p, preferred_element_type=f32)
                acc = o if acc is None else acc + o
        if hp is not None:
            ot_s[hp] = acc * pl.reciprocal(jnp.sum(ls, axis=0, keepdims=True), approx=False)
        if hq is not None:
            return jnp.broadcast_to(jnp.max(mx, axis=0, keepdims=True), (8, BQ))
        return None

    m0 = stage(0, sa, None, None, None)
    def body(j, m):
        for u in range(0, U, 2):
            h = U * j + u
            m = stage(h + 1, sb, h, sa, m)
            m = stage(h + 2, sa, h + 1, sb, m)
        return m
    m = jax.lax.fori_loop(0, H // U - 1, body, m0)
    for h in range(H - U, H - 2, 2):
        m = stage(h + 1, sb, h, sa, m)
        m = stage(h + 2, sa, h + 1, sb, m)
    m = stage(H - 1, sb, H - 2, sa, m)
    stage(None, None, H - 1, sb, m)
    @pl.when(i == 0)
    def _():
        for c in wc[1:]:
            c.wait()
    o = ot_s[...].reshape(D, BQ).T.astype(bf16)
    xn = xn_s[pl.ds(q0, BQ), :]
    a = jnp.dot(o, wo_ref[...], preferred_element_type=f32)
    gt = jnp.dot(xn, wg_ref[...], preferred_element_type=f32)
    up = jnp.dot(xn, wu_ref[...], preferred_element_type=f32)
    hcur = (gt * (1.0 / (1.0 + jnp.exp(-gt))) * up).astype(bf16)
    b = jnp.dot(hcur, wd_ref[...], preferred_element_type=f32)
    o_ref[...] = (x_ref[pl.ds(q0, BQ), :].astype(f32) + a + b).astype(o_ref.dtype)

@jax.jit
def pallas_parallel_sum__mha_block__swiglu_ffn__prompt_kernel(A_x, A_wqkv, A_wo, B_x, B_w_gate, B_w_up, B_w_down):
    x = A_x.reshape(S, D)
    out = pl.pallas_call(
        kern, grid=(S // BQ,),
        in_specs=[pl.BlockSpec(memory_space=pl.ANY)] * 6,
        out_specs=pl.BlockSpec((BQ, D), lambda i: (i, 0)),
        out_shape=jax.ShapeDtypeStruct((S, D), A_x.dtype),
        scratch_shapes=[pltpu.VMEM(a.shape, bf16) for a in (x, A_wqkv, A_wo, B_w_gate, B_w_up, B_w_down)] + [pltpu.VMEM((S, D), bf16), pltpu.VMEM((H, S // 2, DH), jnp.int32), pltpu.VMEM((H, DH, S), bf16),
                        pltpu.VMEM((H, 8, S), jnp.int32), pltpu.VMEM((H, DH, BQ), f32), pltpu.VMEM((S, BQ), f32), pltpu.VMEM((S, BQ), f32),
                        pltpu.SemaphoreType.DMA((S // R,)), pltpu.SemaphoreType.DMA((5,))],
        compiler_params=pltpu.CompilerParams(dimension_semantics=("arbitrary",), vmem_limit_bytes=100 * 1024 * 1024),
    )(x, A_wqkv, A_wo, B_w_gate, B_w_up, B_w_down)
    return out.reshape(1, S, D)
```
